```python
import os as _os
_os.environ.setdefault("JAX_PLATFORMS", "cpu")
import jax
import jax.numpy as jnp

def _softmax(x, axis=-1):
    return jax.nn.softmax(x, axis=axis)
def _gelu(x):
    return jax.nn.gelu(x, approximate=True)
def _silu(x):
    return jax.nn.silu(x)
def _sigmoid(x):
    return jax.nn.sigmoid(x)
def _layernorm(x, axis=-1, eps=1e-5):
    m = jnp.mean(x, axis=axis, keepdims=True)
    v = jnp.var(x, axis=axis, keepdims=True)
    return (x - m) / jnp.sqrt(v + eps)
def _scatter_add(tgt, idx, src, axis=0):
    return tgt.at[idx].add(src)
def _segment_sum(src, seg, n):
    return jax.ops.segment_sum(src, seg, n)
class _Rng:
    def __init__(self, key):
        self._k = key
    def _next(self):
        self._k, sub = jax.random.split(self._k)
        return sub
    def normal(self, shape):
        return jax.random.normal(self._next(), shape, dtype=jnp.bfloat16)
    def randint(self, lo, hi, shape):
        return jax.random.randint(self._next(), shape, lo, hi, dtype=jnp.int32)
    def uniform(self, shape, lo=0.0, hi=1.0):
        return jax.random.uniform(self._next(), shape, jnp.bfloat16, lo, hi)
    def permutation(self, n):
        return jax.random.permutation(self._next(), n)


kernel_name = 'recurrent_scan__sliding_block__dense_activation_mish__prompt'

def setup_inputs():
    _rng = _Rng(jax.random.key(int.from_bytes(__import__("os").urandom(4), "little")))
    _w = (lambda a: (lambda t: t.astype(jnp.bfloat16) if jnp.issubdtype(t.dtype, jnp.floating) else t)(jnp.asarray(a)))
    def _A_setup():
        B, S, D = 1, 2048, 576
        return {
            "x": _w((lambda *s: _rng.normal(s) * 0.05)(B, S, D)),
            "wqkv": _w((lambda *s: _rng.normal(s) * 0.1)(D, 3 * D)),
            "wo": _w((lambda *s: _rng.normal(s) * 0.1)(D, D)),
        }
    _A_in = _A_setup()

    def _B_setup():
        B, S, D, F = 1, 2048, 576, 4608
        return {
            "x": _w((lambda *s: _rng.normal(s) * 0.05)(B, S, D)),
            "w1": _w((lambda *s: _rng.normal(s) * 0.05)(D, F) * (D ** -0.5)),
            "b1": _w((lambda *s: _rng.normal(s) * 0.05)(F)),
            "w2": _w((lambda *s: _rng.normal(s) * 0.05)(F, D) * (F ** -0.5)),
        }
    _B_in = _B_setup()

    return {
        "A_x": _A_in["x"],
        "A_wqkv": _A_in["wqkv"],
        "A_wo": _A_in["wo"],
        "B_x": _B_in["x"],
        "B_w1": _B_in["w1"],
        "B_b1": _B_in["b1"],
        "B_w2": _B_in["w2"],
    }

def reference(A_x, A_wqkv, A_wo, B_x, B_w1, B_b1, B_w2):
    def _A_ref(x, wqkv, wo):
        B, S, D = x.shape
        H = 32; Dh = D // H; W = 256
        qkv = (lambda x, *d: x.transpose(*d))((x @ wqkv).reshape(B, S, 3, H, Dh), 2, 0, 3, 1, 4)
        q, k, v = qkv[0], qkv[1], qkv[2]
        scores = jnp.einsum("bhqd,bhkd->bhqk", q, k) * (Dh ** -0.5)
        idx = jnp.arange(S)
        mask = (idx[:, None] - idx[None, :] >= 0) & (idx[:, None] - idx[None, :] < W)
        scores = jnp.where(mask[None, None], scores, -1e9)
        p = _softmax(scores, axis=-1)
        o = jnp.einsum("bhqk,bhkd->bhqd", p, v)
        return (lambda x, *d: x.transpose(*d))(o, 0, 2, 1, 3).reshape(B, S, D) @ wo

    def _B_ref(x, w1, b1, w2):
        h = jnp.einsum("bsd,df->bsf", x, w1) + b1
        sp = jnp.log1p(jnp.exp(-jnp.abs(h))) + jnp.where(h > 0, h, jnp.zeros_like(h))
        act = h * jnp.tanh(sp)
        return jnp.einsum("bsf,fd->bsd", act, w2)

    x = A_x
    xn = _layernorm(x, axis=-1)
    s = _A_ref(xn, A_wqkv, A_wo)
    g = _silu(_B_ref(xn, B_w1, B_b1, B_w2))
    return x + s * g
```

```python
import jax
import jax.numpy as jnp
from jax import lax
import jax.experimental.pallas as pl
import jax.experimental.pallas.tpu as pltpu

S, D, F, H, DH, WIN = 2048, 576, 4608, 32, 18, 256
TQ = 128
DP = 640
NB = S // TQ
G = 8
GW = 4 * DH
NTL = F // 128
PC = 384
DEFER = 256
NEG = -1e9
LOG2E = 1.4426950408889634
BF, F32 = jnp.bfloat16, jnp.float32
NT = (((1,), (1,)), ((), ()))


def _row0(i):
    return i * TQ if isinstance(i, int) else pl.multiple_of(i * TQ, TQ)


def _kernel(x_hbm, wqkv_hbm, wo_hbm, w1_hbm, b1_hbm, w2t_hbm, o_hbm,
            x_v, wqk_v, wv_v, wo_v, w1_v, b1_v, w2t_v, wvt_v, wot_v,
            xn_v, q_v, k_v, vt_v, out_v, xnt_v, acc_v, actl_v, sems, osem, xsem):
    def xcopy(i):
        r0 = _row0(i)
        return pltpu.make_async_copy(x_hbm.at[:, pl.ds(r0, TQ)], x_v.at[:, pl.ds(r0, TQ)], xsem.at[i])

    def ocopy(i):
        r0 = _row0(i)
        return pltpu.make_async_copy(out_v.at[:, pl.ds(r0, TQ)], o_hbm.at[:, pl.ds(r0, TQ)], osem.at[i])

    cv = pltpu.make_async_copy(wqkv_hbm.at[:, 2 * D:3 * D], wv_v, sems.at[0])
    cqk = pltpu.make_async_copy(wqkv_hbm.at[:, 0:2 * D], wqk_v, sems.at[1])
    cwo = pltpu.make_async_copy(wo_hbm, wo_v, sems.at[2])
    cw2 = pltpu.make_async_copy(w2t_hbm, w2t_v, sems.at[3])
    cw1 = pltpu.make_async_copy(w1_hbm, w1_v, sems.at[4])
    cb1 = pltpu.make_async_copy(b1_hbm, b1_v, sems.at[5])
    xcopy(0).start(); cv.start(); cqk.start(); xcopy(1).start()

    def ln(i):
        r0 = _row0(i)
        x = x_v[:, pl.ds(r0, TQ)].astype(F32)
        m = jnp.sum(x, axis=0, keepdims=True) * (1.0 / D)
        xc = x - m
        var = jnp.sum(xc * xc, axis=0, keepdims=True) * (1.0 / D)
        xnt = (xc * lax.rsqrt(var + 1e-5)).astype(BF)
        xnt_v[i] = xnt
        xn_v[pl.ds(r0, TQ), :] = jnp.concatenate([xnt, jnp.zeros((DP - D, TQ), BF)], axis=0).T

    xcopy(0).wait()
    ln(0)
    cv.wait()
    wvt_v[...] = wv_v[...].T
    cqk.wait()
    for i in range(2, NB):
        xcopy(i).start()
    cwo.start(); cb1.start(); cw1.start(); cw2.start()

    def proj(i):
        r0 = _row0(i)
        xn = xn_v[pl.ds(r0, TQ), 0:D]
        lane = lax.broadcasted_iota(jnp.int32, (TQ, 128), 1)
        ones = jnp.ones((8, TQ), F32)
        tiles = {}

        def mm(c):
            r = jnp.dot(xn, wqk_v[:, c * PC:(c + 1) * PC], preferred_element_type=F32)
            for k in range(PC // 128):
                tiles[c * PC // 128 + k] = r[:, 128 * k:128 * k + 128]

        def cols(col):
            t0, t1 = col // 128, min((col + 127) // 128, 2 * D // 128 - 1)
            for t in (t0, t1):
                while t not in tiles:
                    mm(len(tiles) * 128 // PC)
            o = col % 128
            if o == 0:
                return tiles[t0]
            if t0 == t1:
                return pltpu.roll(tiles[t0], 128 - o, 1)
            return pltpu.roll(jnp.where(lane >= o, tiles[t0], tiles[t1]), 128 - o, 1)

        vt = jnp.dot(wvt_v[...], xnt_v[i], preferred_element_type=F32)
        mm(0)
        for g in range(G):
            vt_v[i, 2 * g] = jnp.concatenate([vt[g * GW:g * GW + 40], ones], axis=0).astype(BF)
            vt_v[i, 2 * g + 1] = jnp.concatenate([vt[g * GW + 32:g * GW + 72], ones], axis=0).astype(BF)
        for g in range(G):
            if g == 2 and not (isinstance(i, int) and i == NB - 1):
                ln(i + 1)
            q_v[g, pl.ds(r0, TQ), :] = (cols(g * GW) * (DH ** -0.5 * LOG2E)).astype(BF)
        for g in range(G):
            k_v[g, pl.ds(r0, TQ), :] = cols(D + g * GW).astype(BF)

    def proj2(ii, _):
        for k in range(2):
            xcopy(ii * 2 + k + 2).wait()
        for k in range(2):
            proj(ii * 2 + k + 1)
        return 0

    xcopy(1).wait()
    proj(0)
    lax.fori_loop(0, (NB - 2) // 2, proj2, 0)
    cwo.wait()
    wot_v[...] = wo_v[...].T
    proj(NB - 1)
    cb1.wait(); cw1.wait(); cw2.wait()

    def epilogue(i):
        r0 = _row0(i)
        st = acc_v[0]
        gt = acc_v[1] + lax.dot_general(w2t_v[:, F - DEFER:F], actl_v[...], NT, preferred_element_type=F32)
        z = st * gt * pltpu.reciprocal(1.0 + jnp.exp(-gt), approx=True)
        out_v[:, pl.ds(r0, TQ)] = (x_v[:, pl.ds(r0, TQ)].astype(F32) + z).astype(BF)

    def block(i, _):
        head = isinstance(i, int)
        r0 = _row0(i)
        xn = xn_v[pl.ds(r0, TQ), 0:D]
        row = lax.broadcasted_iota(jnp.int32, (64, 128), 0)
        col = lax.broadcasted_iota(jnp.int32, (64, 128), 1)
        m_first = row > (col & 63)
        l32 = lax.broadcasted_iota(jnp.int32, (32, 128), 1)
        r40 = lax.broadcasted_iota(jnp.int32, (40, 128), 0)
        c40 = lax.broadcasted_iota(jnp.int32, (40, 128), 1)
        r8 = lax.broadcasted_iota(jnp.int32, (8, 128), 0)

        def scores(g, p, j):
            h0 = 2 * p * DH
            q = pltpu.bitcast(q_v[g, pl.ds(r0 + 64 * j, 64), :], jnp.int32)
            qa = jnp.where((l32 >= h0) & (l32 < h0 + DH), q, 0)
            qb = jnp.where((l32 >= h0 + DH) & (l32 < h0 + 2 * DH), q, 0)
            qbd = pltpu.bitcast(jnp.concatenate([qa, qb], axis=0), BF)
            if head:
                kw = k_v[g, 0:r0 + 64 * j + 64, :]
            else:
                kw = k_v[g, pl.ds(r0 + 64 * j - WIN, WIN + 64), :]
            return lax.dot_general(kw, qbd, NT, preferred_element_type=F32)

        def softmax(st):
            if head:
                n = st.shape[0] - 64
                st = jnp.concatenate(([st[0:n]] if n else []) + [jnp.where(m_first, NEG, st[n:])], axis=0)
                return jnp.exp2(st - jnp.max(st, axis=0, keepdims=True)).astype(BF)
            st = jnp.concatenate([jnp.where(m_first, st[0:64], st[WIN:]), st[64:WIN]], axis=0)
            e = jnp.exp2(st - jnp.max(st, axis=0, keepdims=True))
            return jnp.concatenate([jnp.where(m_first, e[0:64], 0.0), e[64:WIN],
                                    jnp.where(m_first, 0.0, e[0:64])], axis=0).astype(BF)

        def pv(g, p, j, pt):
            if head:
                vt = jnp.concatenate([vt_v[t, 2 * g + p] for t in range(i + 1)], axis=1)[:, 0:pt.shape[0]]
            else:
                vt = jnp.concatenate([vt_v[i - 2 + t, 2 * g + p] for t in range(3)], axis=1)
                vt = vt[:, 64 * j:64 * j + WIN + 64]
            ot = jnp.dot(vt, pt, preferred_element_type=F32)
            return ot[0:40] * pltpu.reciprocal(ot[40:41], approx=True)

        def merge(o):
            outs = []
            for p in range(2):
                a, b = o[2 * p], o[2 * p + 1]
                first = r40 < (DH + 4 * p)
                e = pltpu.roll(jnp.where(first, b, a), 64, 1)
                outs.append(jnp.where(first == (c40 < 64), jnp.where(first, a, b), e))
            mid = jnp.where(r8 < 4, outs[0][32:40], outs[1][0:8])
            return jnp.concatenate([outs[0][0:32], mid, outs[1][8:40]], axis=0)

        def f1(c):
            h = jnp.dot(xn, w1_v[:, c * 128:(c + 1) * 128], preferred_element_type=F32)
            return h + b1_v[c:c + 1, :].astype(F32)

        def mish(h):
            n = jnp.exp2(jnp.minimum(h, 20.0) * LOG2E)
            t = n * (n + 2.0)
            return (h * t * pltpu.reciprocal(t + 2.0, approx=True)).astype(BF)

        def f2(c, act):
            return lax.dot_general(w2t_v[:, c * 256:(c + 1) * 256], act, NT, preferred_element_type=F32)

        units = [(g, p, j) for g in range(G) for p in range(2) for j in range(2)]
        ss, hs, ps, acts, os_, ots = {}, {}, {}, {}, {}, []
        gt = None
        for t in range(-1, NTL + 1):
            if t + 1 < len(units):
                ss[t + 1] = scores(*units[t + 1])
            if t + 1 < NTL:
                hs[t + 1] = f1(t + 1)
            if t == -1 and not (head and i == 0):
                epilogue(i - 1)
            if 0 <= t < len(units):
                ps[t] = softmax(ss.pop(t))
            if 0 <= t < NTL:
                acts[t] = mish(hs.pop(t))
            u = t - 1
            if 0 <= u < len(units):
                os_[u] = pv(*units[u], ps.pop(u))
                if u % 4 == 3:
                    ots.append(merge([os_.pop(u - 3 + k) for k in range(4)]))
            u = t - 2
            if 0 <= u < NTL - DEFER // 128 and u % 2 == 1:
                y = f2(u // 2, jnp.concatenate([acts.pop(u - 1), acts.pop(u)], axis=1))
                gt = y if gt is None else gt + y
        actl_v[...] = jnp.concatenate([acts.pop(k) for k in range(NTL - DEFER // 128, NTL)], axis=1)
        acc_v[0] = jnp.dot(wot_v[...], jnp.concatenate(ots, axis=0).astype(BF), preferred_element_type=F32)
        acc_v[1] = gt
        if not (head and i == 0):
            ocopy(i - 1).start()
        return 0

    block(0, 0)
    block(1, 0)
    lax.fori_loop(2, NB, block, 0)
    epilogue(NB - 1)
    ocopy(NB - 1).start()
    for i in range(NB):
        ocopy(i).wait()


@jax.jit
def pallas_recurrent_scan__sliding_block__dense_activation_mish__prompt_kernel(
    A_x: jax.Array,
    A_wqkv: jax.Array,
    A_wo: jax.Array,
    B_x: jax.Array,
    B_w1: jax.Array,
    B_b1: jax.Array,
    B_w2: jax.Array,
):
    hbm = pl.BlockSpec(memory_space=pltpu.MemorySpace.HBM)
    out = pl.pallas_call(
        _kernel,
        out_shape=pltpu.MemorySpace.HBM((D, S), BF),
        in_specs=[hbm] * 6,
        out_specs=hbm,
        scratch_shapes=[
            pltpu.VMEM((D, S), BF),
            pltpu.VMEM((D, 2 * D), BF),
            pltpu.VMEM((D, D), BF),
            pltpu.VMEM((D, D), BF),
            pltpu.VMEM((D, F), BF),
            pltpu.VMEM((NTL, 128), BF),
            pltpu.VMEM((D, F), BF),
            pltpu.VMEM((D, D), BF),
            pltpu.VMEM((D, D), BF),
            pltpu.VMEM((S, DP), BF),
            pltpu.VMEM((G, S, 128), BF),
            pltpu.VMEM((G, S, 128), BF),
            pltpu.VMEM((NB, 2 * G, 48, TQ), BF),
            pltpu.VMEM((D, S), BF),
            pltpu.VMEM((NB, D, TQ), BF),
            pltpu.VMEM((2, D, TQ), F32),
            pltpu.VMEM((TQ, DEFER), BF),
            pltpu.SemaphoreType.DMA((6,)),
            pltpu.SemaphoreType.DMA((NB,)),
            pltpu.SemaphoreType.DMA((NB,)),
        ],
        compiler_params=pltpu.CompilerParams(vmem_limit_bytes=100 * 2**20),
        name="fused",
    )(A_x.reshape(S, D).T, A_wqkv, A_wo, B_w1, B_b1.reshape(NTL, 128), B_w2.T)
    return out.T.reshape(1, S, D)
```

```python
import jax
import jax.numpy as jnp
from jax import lax
import jax.experimental.pallas as pl
import jax.experimental.pallas.tpu as pltpu

S, D, F, H, DH, WIN = 2048, 576, 4608, 32, 18, 256
TQ = 128
DP = 640
NB = S // TQ
G = 8
GW = 4 * DH
NTL = F // 128
PC = 384
DEFER = 256
NEG = -1e9
LOG2E = 1.4426950408889634
BF, F32 = jnp.bfloat16, jnp.float32
NT = (((1,), (1,)), ((), ()))


def _row0(i):
    return i * TQ if isinstance(i, int) else pl.multiple_of(i * TQ, TQ)


def _kernel(x_hbm, wqkv_hbm, wo_hbm, w1_hbm, b1_hbm, w2t_hbm, o_hbm,
            x_v, wqk_v, wv_v, wo_v, w1_v, b1_v, w2t_v, wvt_v, wot_v,
            xn_v, q_v, k_v, vt_v, out_v, xnt_v, acc_v, actl_v, sems, osem, xsem):
    def xcopy(i):
        r0 = _row0(i)
        return pltpu.make_async_copy(x_hbm.at[:, pl.ds(r0, TQ)], x_v.at[:, pl.ds(r0, TQ)], xsem.at[i])

    def ocopy(i):
        r0 = _row0(i)
        return pltpu.make_async_copy(out_v.at[:, pl.ds(r0, TQ)], o_hbm.at[:, pl.ds(r0, TQ)], osem.at[i])

    cv = pltpu.make_async_copy(wqkv_hbm.at[:, 2 * D:3 * D], wv_v, sems.at[0])
    cqk = pltpu.make_async_copy(wqkv_hbm.at[:, 0:2 * D], wqk_v, sems.at[1])
    cwo = pltpu.make_async_copy(wo_hbm, wo_v, sems.at[2])
    cw2 = pltpu.make_async_copy(w2t_hbm, w2t_v, sems.at[3])
    cw1 = pltpu.make_async_copy(w1_hbm, w1_v, sems.at[4])
    cb1 = pltpu.make_async_copy(b1_hbm, b1_v, sems.at[5])
    xcopy(0).start(); cv.start(); xcopy(1).start(); cqk.start()

    def ln(i):
        r0 = _row0(i)
        x = x_v[:, pl.ds(r0, TQ)].astype(F32)
        m = jnp.sum(x, axis=0, keepdims=True) * (1.0 / D)
        xc = x - m
        var = jnp.sum(xc * xc, axis=0, keepdims=True) * (1.0 / D)
        xnt = (xc * lax.rsqrt(var + 1e-5)).astype(BF)
        xnt_v[i] = xnt
        xn_v[pl.ds(r0, TQ), :] = jnp.concatenate([xnt, jnp.zeros((DP - D, TQ), BF)], axis=0).T

    xcopy(0).wait()
    ln(0)
    cv.wait()
    wvt_v[...] = wv_v[...].T

    def vproj(i):
        vt = jnp.dot(wvt_v[...], xnt_v[i], preferred_element_type=F32)
        ones = jnp.ones((8, TQ), F32)
        for g in range(G):
            vt_v[i, 2 * g] = jnp.concatenate([vt[g * GW:g * GW + 40], ones], axis=0).astype(BF)
            vt_v[i, 2 * g + 1] = jnp.concatenate([vt[g * GW + 32:g * GW + 72], ones], axis=0).astype(BF)

    def proj(i, with_v=True, next_ln=True):
        r0 = _row0(i)
        xn = xn_v[pl.ds(r0, TQ), 0:D]
        lane = lax.broadcasted_iota(jnp.int32, (TQ, 128), 1)
        tiles = {}

        def mm(c):
            r = jnp.dot(xn, wqk_v[:, c * PC:(c + 1) * PC], preferred_element_type=F32)
            for k in range(PC // 128):
                tiles[c * PC // 128 + k] = r[:, 128 * k:128 * k + 128]

        def cols(col):
            t0, t1 = col // 128, min((col + 127) // 128, 2 * D // 128 - 1)
            for t in (t0, t1):
                while t not in tiles:
                    mm(len(tiles) * 128 // PC)
            o = col % 128
            if o == 0:
                return tiles[t0]
            if t0 == t1:
                return pltpu.roll(tiles[t0], 128 - o, 1)
            return pltpu.roll(jnp.where(lane >= o, tiles[t0], tiles[t1]), 128 - o, 1)

        if with_v:
            vproj(i)
        mm(0)
        for g in range(G):
            if g == 2 and next_ln:
                ln(i + 1)
            q_v[g, pl.ds(r0, TQ), :] = (cols(g * GW) * (DH ** -0.5 * LOG2E)).astype(BF)
        for g in range(G):
            k_v[g, pl.ds(r0, TQ), :] = cols(D + g * GW).astype(BF)

    def proj2(ii, _):
        for k in range(2):
            xcopy(ii * 2 + k + 3).wait()
        for k in range(2):
            proj(ii * 2 + k + 2)
        return 0

    xcopy(1).wait()
    ln(1)
    vproj(0)
    vproj(1)
    cqk.wait()
    for i in range(2, NB):
        xcopy(i).start()
    cwo.start(); cb1.start(); cw1.start(); cw2.start()
    proj(0, False, False)
    xcopy(2).wait()
    proj(1, False)
    lax.fori_loop(0, (NB - 4) // 2, proj2, 0)
    xcopy(NB - 1).wait()
    cwo.wait()
    wot_v[...] = wo_v[...].T
    proj(NB - 2)
    proj(NB - 1, True, False)
    cb1.wait(); cw1.wait(); cw2.wait()

    def epilogue(i):
        r0 = _row0(i)
        st = acc_v[0]
        gt = acc_v[1] + lax.dot_general(w2t_v[:, F - DEFER:F], actl_v[...], NT, preferred_element_type=F32)
        z = st * gt * pltpu.reciprocal(1.0 + jnp.exp(-gt), approx=True)
        out_v[:, pl.ds(r0, TQ)] = (x_v[:, pl.ds(r0, TQ)].astype(F32) + z).astype(BF)

    def block(i, _):
        head = isinstance(i, int)
        r0 = _row0(i)
        xn = xn_v[pl.ds(r0, TQ), 0:D]
        row = lax.broadcasted_iota(jnp.int32, (64, 128), 0)
        col = lax.broadcasted_iota(jnp.int32, (64, 128), 1)
        m_first = row > (col & 63)
        l32 = lax.broadcasted_iota(jnp.int32, (32, 128), 1)
        r40 = lax.broadcasted_iota(jnp.int32, (40, 128), 0)
        c40 = lax.broadcasted_iota(jnp.int32, (40, 128), 1)
        r8 = lax.broadcasted_iota(jnp.int32, (8, 128), 0)

        def scores(g, p, j):
            h0 = 2 * p * DH
            q = pltpu.bitcast(q_v[g, pl.ds(r0 + 64 * j, 64), :], jnp.int32)
            qa = jnp.where((l32 >= h0) & (l32 < h0 + DH), q, 0)
            qb = jnp.where((l32 >= h0 + DH) & (l32 < h0 + 2 * DH), q, 0)
            qbd = pltpu.bitcast(jnp.concatenate([qa, qb], axis=0), BF)
            if head:
                kw = k_v[g, 0:r0 + 64 * j + 64, :]
            else:
                kw = k_v[g, pl.ds(r0 + 64 * j - WIN, WIN + 64), :]
            return lax.dot_general(kw, qbd, NT, preferred_element_type=F32)

        def softmax(st):
            if head:
                n = st.shape[0] - 64
                st = jnp.concatenate(([st[0:n]] if n else []) + [jnp.where(m_first, NEG, st[n:])], axis=0)
                return jnp.exp2(st - jnp.max(st, axis=0, keepdims=True)).astype(BF)
            st = jnp.concatenate([jnp.where(m_first, st[0:64], st[WIN:]), st[64:WIN]], axis=0)
            e = jnp.exp2(st - jnp.max(st, axis=0, keepdims=True))
            return jnp.concatenate([jnp.where(m_first, e[0:64], 0.0), e[64:WIN],
                                    jnp.where(m_first, 0.0, e[0:64])], axis=0).astype(BF)

        def pv(g, p, j, pt):
            if head:
                vt = jnp.concatenate([vt_v[t, 2 * g + p] for t in range(i + 1)], axis=1)[:, 0:pt.shape[0]]
            else:
                vt = jnp.concatenate([vt_v[i - 2 + t, 2 * g + p] for t in range(3)], axis=1)
                vt = vt[:, 64 * j:64 * j + WIN + 64]
            ot = jnp.dot(vt, pt, preferred_element_type=F32)
            return ot[0:40] * pltpu.reciprocal(ot[40:41], approx=True)

        def merge(o):
            outs = []
            for p in range(2):
                a, b = o[2 * p], o[2 * p + 1]
                first = r40 < (DH + 4 * p)
                e = pltpu.roll(jnp.where(first, b, a), 64, 1)
                outs.append(jnp.where(first == (c40 < 64), jnp.where(first, a, b), e))
            mid = jnp.where(r8 < 4, outs[0][32:40], outs[1][0:8])
            return jnp.concatenate([outs[0][0:32], mid, outs[1][8:40]], axis=0)

        def f1(c):
            h = jnp.dot(xn, w1_v[:, c * 128:(c + 1) * 128], preferred_element_type=F32)
            return h + b1_v[c:c + 1, :].astype(F32)

        def mish(h):
            n = jnp.exp2(jnp.minimum(h, 20.0) * LOG2E)
            t = n * (n + 2.0)
            return (h * t * pltpu.reciprocal(t + 2.0, approx=True)).astype(BF)

        def f2(c, act):
            return lax.dot_general(w2t_v[:, c * 256:(c + 1) * 256], act, NT, preferred_element_type=F32)

        units = [(g, p, j) for g in range(G) for p in range(2) for j in range(2)]
        ss, hs, ps, acts, os_, ots = {}, {}, {}, {}, {}, []
        gt = None
        for t in range(-1, NTL + 1):
            if t + 1 < len(units):
                ss[t + 1] = scores(*units[t + 1])
            if t + 1 < NTL:
                hs[t + 1] = f1(t + 1)
            if t == -1 and not (head and i == 0):
                epilogue(i - 1)
            if 0 <= t < len(units):
                ps[t] = softmax(ss.pop(t))
            if 0 <= t < NTL:
                acts[t] = mish(hs.pop(t))
            u = t - 1
            if 0 <= u < len(units):
                os_[u] = pv(*units[u], ps.pop(u))
                if u % 4 == 3:
                    ots.append(merge([os_.pop(u - 3 + k) for k in range(4)]))
            u = t - 2
            if 0 <= u < NTL - DEFER // 128 and u % 2 == 1:
                y = f2(u // 2, jnp.concatenate([acts.pop(u - 1), acts.pop(u)], axis=1))
                gt = y if gt is None else gt + y
        actl_v[...] = jnp.concatenate([acts.pop(k) for k in range(NTL - DEFER // 128, NTL)], axis=1)
        acc_v[0] = jnp.dot(wot_v[...], jnp.concatenate(ots, axis=0).astype(BF), preferred_element_type=F32)
        acc_v[1] = gt
        if not (head and i == 0):
            ocopy(i - 1).start()
        return 0

    block(0, 0)
    block(1, 0)
    lax.fori_loop(2, NB, block, 0)
    epilogue(NB - 1)
    ocopy(NB - 1).start()
    for i in range(NB):
        ocopy(i).wait()


@jax.jit
def pallas_recurrent_scan__sliding_block__dense_activation_mish__prompt_kernel(
    A_x: jax.Array,
    A_wqkv: jax.Array,
    A_wo: jax.Array,
    B_x: jax.Array,
    B_w1: jax.Array,
    B_b1: jax.Array,
    B_w2: jax.Array,
):
    hbm = pl.BlockSpec(memory_space=pltpu.MemorySpace.HBM)
    out = pl.pallas_call(
        _kernel,
        out_shape=pltpu.MemorySpace.HBM((D, S), BF),
        in_specs=[hbm] * 6,
        out_specs=hbm,
        scratch_shapes=[
            pltpu.VMEM((D, S), BF),
            pltpu.VMEM((D, 2 * D), BF),
            pltpu.VMEM((D, D), BF),
            pltpu.VMEM((D, D), BF),
            pltpu.VMEM((D, F), BF),
            pltpu.VMEM((NTL, 128), BF),
            pltpu.VMEM((D, F), BF),
            pltpu.VMEM((D, D), BF),
            pltpu.VMEM((D, D), BF),
            pltpu.VMEM((S, DP), BF),
            pltpu.VMEM((G, S, 128), BF),
            pltpu.VMEM((G, S, 128), BF),
            pltpu.VMEM((NB, 2 * G, 48, TQ), BF),
            pltpu.VMEM((D, S), BF),
            pltpu.VMEM((NB, D, TQ), BF),
            pltpu.VMEM((2, D, TQ), F32),
            pltpu.VMEM((TQ, DEFER), BF),
            pltpu.SemaphoreType.DMA((6,)),
            pltpu.SemaphoreType.DMA((NB,)),
            pltpu.SemaphoreType.DMA((NB,)),
        ],
        compiler_params=pltpu.CompilerParams(vmem_limit_bytes=100 * 2**20),
        name="fused",
    )(A_x.reshape(S, D).T, A_wqkv, A_wo, B_w1, B_b1.reshape(NTL, 128), B_w2.T)
    return out.T.reshape(1, S, D)
```
